```python
import jax
import jax.numpy as jnp

def _softmax(x, axis=-1):
    return jax.nn.softmax(x, axis=axis)

def _gelu(x):
    return jax.nn.gelu(x, approximate=True)

def _silu(x):
    return jax.nn.silu(x)

def _sigmoid(x):
    return jax.nn.sigmoid(x)

def _layernorm(x, axis=-1, eps=1e-05):
    m = jnp.mean(x, axis=axis, keepdims=True)
    v = jnp.var(x, axis=axis, keepdims=True)
    return (x - m) / jnp.sqrt(v + eps)

def _scatter_add(tgt, idx, src, axis=0):
    return tgt.at[idx].add(src)

def _segment_sum(src, seg, n):
    return jax.ops.segment_sum(src, seg, n)

class _Rng:

    def __init__(self, key):
        self._k = key

    def _next(self):
        self._k, sub = jax.random.split(self._k)
        return sub

    def normal(self, shape):
        return jax.random.normal(self._next(), shape, dtype=jnp.bfloat16)

    def randint(self, lo, hi, shape):
        return jax.random.randint(self._next(), shape, lo, hi, dtype=jnp.int32)

    def uniform(self, shape, lo=0.0, hi=1.0):
        return jax.random.uniform(self._next(), shape, jnp.bfloat16, lo, hi)

    def permutation(self, n):
        return jax.random.permutation(self._next(), n)
kernel_name = 'adaLN_cond__mha_block_cached__moe_arch_mod__prompt'

def setup_inputs():
    _rng = _Rng(jax.random.key(int.from_bytes(__import__("os").urandom(4), "little")))
    _w = lambda a: (lambda t: t.astype(jnp.bfloat16) if jnp.issubdtype(t.dtype, jnp.floating) else t)(jnp.asarray(a))

    def _A_setup():
        B, Sq, D = (1, 2048, 1024)
        H, Sk, Dh = (32, 2048, 128)
        return {'x': _w((lambda *s: _rng.normal(s) * 0.05)(B, Sq, D)), 'k_cache': _w((lambda *s: _rng.normal(s) * 0.05)(B, H, Sk, Dh)), 'v_cache': _w((lambda *s: _rng.normal(s) * 0.05)(B, H, Sk, Dh)), 'wq': _w((lambda *s: _rng.normal(s) * 0.05)(D, H * Dh) * D ** (-0.5)), 'wo': _w((lambda *s: _rng.normal(s) * 0.05)(H * Dh, D) * (H * Dh) ** (-0.5))}
    _A_in = _A_setup()

    def _B_setup():
        B, S, D, F, C = (1, 2048, 1024, 3584, 2)
        return {'x': _w((lambda *s: _rng.normal(s) * 0.05)(B, S, D)), 'w_r': _w((lambda *s: _rng.normal(s) * 0.05)(D)), 'w_gate': _w((lambda *s: _rng.normal(s) * 0.05)(D, F)), 'w_up': _w((lambda *s: _rng.normal(s) * 0.05)(D, F)), 'w_down': _w((lambda *s: _rng.normal(s) * 0.05)(F, D))}
    _B_in = _B_setup()
    return {'A_x': _A_in['x'], 'A_k_cache': _A_in['k_cache'], 'A_v_cache': _A_in['v_cache'], 'A_wq': _A_in['wq'], 'A_wo': _A_in['wo'], 'B_x': _B_in['x'], 'B_w_r': _B_in['w_r'], 'B_w_gate': _B_in['w_gate'], 'B_w_up': _B_in['w_up'], 'B_w_down': _B_in['w_down'], 'c': _w((lambda *s: _rng.normal(s) * 0.05)(1, 1024)), 'w_mod': _w((lambda *s: _rng.normal(s) * 0.05)(1024, 6 * 1024) * 1024 ** (-0.5))}

def reference(A_x, A_k_cache, A_v_cache, A_wq, A_wo, B_x, B_w_r, B_w_gate, B_w_up, B_w_down, c, w_mod):

    def _A_ref(x, k_cache, v_cache, wq, wo):
        B, Sq, D = x.shape
        H, Dh = (32, 128)
        q = (lambda x, *d: x.transpose(*d))((x @ wq).reshape(B, Sq, H, Dh), 0, 2, 1, 3)
        scores = jnp.einsum('bhqd,bhkd->bhqk', q, k_cache) * Dh ** (-0.5)
        p = _softmax(scores, axis=-1)
        o = jnp.einsum('bhqk,bhkd->bhqd', p, v_cache)
        return (lambda x, *d: x.transpose(*d))(o, 0, 2, 1, 3).reshape(B, Sq, H * Dh) @ wo

    def _B_ref(x, w_r, w_gate, w_up, w_down):
        B, S, D = x.shape
        C = 2
        r = x @ w_r
        idx = jnp.argsort(-r, axis=-1)[:, :C]
        idx_e = jnp.repeat(idx.reshape(B, C, 1), D, axis=2)
        x_sel = jnp.take_along_axis(x, idx_e, axis=1)
        g = _silu(x_sel @ w_gate)
        u = x_sel @ w_up
        y = g * u @ w_down
        r_sel = _sigmoid(jnp.take_along_axis(r, idx, axis=1))
        y = y * r_sel.reshape(B, C, 1)
        b_off = (jnp.arange(B) * S).reshape(B, 1)
        flat_idx = (idx + b_off).reshape(B * C)
        zero = (x * 0.0).reshape(B * S, D)
        upd = _scatter_add(zero, flat_idx, y.reshape(B * C, D), axis=0)
        return x + upd.reshape(B, S, D)
    x = A_x
    mod = (_silu(c) @ w_mod).reshape(c.shape[0], 6, 1, -1)
    sa, ca, ga, sb, cb, gb = (mod[:, 0].copy(), mod[:, 1].copy(), mod[:, 2].copy(), mod[:, 3].copy(), mod[:, 4].copy(), mod[:, 5].copy())
    h = _layernorm(x, axis=-1) * (1 + ca) + sa
    x = x + ga * _A_ref(h, A_k_cache, A_v_cache, A_wq, A_wo)
    h = _layernorm(x, axis=-1) * (1 + cb) + sb
    x = x + gb * _B_ref(h, B_w_r, B_w_gate, B_w_up, B_w_down)
    return x
```

```python
import jax
import jax.numpy as jnp
import numpy as np
from jax import lax
import jax.experimental.pallas as pl
import jax.experimental.pallas.tpu as pltpu

S, D, H, DH, F = 2048, 1024, 32, 128, 3584
TQ = 256
NT = S // TQ
G = 2
NJ = (H - 2) // G
F32, BF16 = jnp.float32, jnp.bfloat16
QSCALE = float(DH ** -0.5 * np.log2(np.e))
EPS = 1e-5
EPS_B = float(np.asarray(EPS, dtype=np.float32).astype(BF16).astype(np.float32))
NT_DIMS = (((1,), (1,)), ((), ()))


def _rb(x):
    return x.astype(BF16).astype(F32)


def _t(i):
    return slice(i * TQ, (i + 1) * TQ)


def _kernel(c_ref, wr_ref, x_hbm, k_hbm, v_hbm, wq_hbm, wo_hbm, wg_hbm, wu_hbm,
            wd_hbm, wm_hbm, out_hbm,
            x_v, h_v, k_v, v_v, wq_v, wo_v, acc_v, os_v, ls_v, q_v, mod_v,
            sem_x, sem_k, sem_v, sem_q, sem_o):

    def x_copy(i):
        return pltpu.make_async_copy(x_hbm.at[0, _t(i)], x_v.at[_t(i)], sem_x.at[i])

    def kv_copy(hbm, vm, sem, j, h0, n):
        return pltpu.make_async_copy(hbm.at[0, pl.ds(h0, n)], vm.at[pl.ds(h0, n)], sem.at[j])

    def wq_copy(g):
        cols = pl.ds(pl.multiple_of(g * 2 * DH, 2 * DH), 2 * DH)
        return pltpu.make_async_copy(wq_hbm.at[:, cols], wq_v.at[g], sem_q.at[g])

    def wo_copy(g):
        r_ = pl.ds(pl.multiple_of(g * 2 * DH, 2 * DH), 2 * DH)
        return pltpu.make_async_copy(wo_hbm.at[r_], wo_v.at[r_], sem_o.at[g])

    def iter_copies(j):
        cps = [kv_copy(k_hbm, k_v, sem_k, j, G * j + 1, G),
               kv_copy(v_hbm, v_v, sem_v, j, G * j + 1, G)]
        for e in range(G // 2):
            cps.append(wq_copy(j * (G // 2) + e + 1))
            cps.append(wo_copy(j * (G // 2) + e))
        return cps

    edge_copies = lambda j, h: [kv_copy(k_hbm, k_v, sem_k, j, h, 1),
                                kv_copy(v_hbm, v_v, sem_v, j, h, 1)]
    first_kv = edge_copies(NJ, 0)
    last_copies = edge_copies(NJ + 1, H - 1) + [wo_copy(H // 2 - 1)]

    def q_proj(g, e, par, i):
        q = jnp.dot(h_v[_t(i), :], wq_v[g, :, e * DH:(e + 1) * DH],
                    preferred_element_type=F32)
        q_v[par, _t(i), :] = (q * QSCALE).astype(BF16)

    def qk(h, par, i):
        return lax.dot_general(q_v[par, _t(i), :], k_v[h], NT_DIMS,
                               preferred_element_type=F32)

    def pv(h, i, s):
        m = jnp.max(s, axis=-1, keepdims=True)
        p = jnp.exp2(s - m)
        l = p[:, 0:128]
        for j in range(1, S // 128):
            l = l + p[:, j * 128:(j + 1) * 128]
        os_v[_t(i), :] = jnp.dot(p.astype(BF16), v_v[h], preferred_element_type=F32)
        ls_v[_t(i), :] = l

    def out_proj(h, i):
        l = jnp.sum(ls_v[_t(i), :], axis=-1, keepdims=True)
        r0 = pltpu.reciprocal(l, approx=True)
        inv = r0 * (2.0 - l * r0)
        o = (os_v[_t(i), :] * inv).astype(BF16)
        r_ = pl.ds(pl.multiple_of(h * DH, DH), DH)
        return jnp.dot(o, wo_v[r_, :], preferred_element_type=F32)

    def run_head(seq, h, par, g_next=None, e_next=None):
        ss = {}
        for tok in seq.split():
            kind, i = tok[0], int(tok[1:])
            if kind == 'Q':
                ss[i] = qk(h, par, i)
            elif kind == 'P':
                pv(h, i, ss.pop(i))
            elif kind == 'N':
                acc_v[_t(i), :] += out_proj(h - 1, i)
            elif kind == 'X':
                q_proj(g_next, e_next, 1 - par, i)

    def prologue(wm_v, sem_m):
        def m_copy(j):
            return pltpu.make_async_copy(wm_hbm.at[:, j * D:(j + 1) * D], wm_v.at[j], sem_m.at[j])

        x_copy(0).start()
        m_copy(0).start()
        m_copy(1).start()
        wq_copy(0).start()
        for i in range(1, NT):
            x_copy(i).start()
        for cp in first_kv:
            cp.start()
        for j in range(2, 6):
            m_copy(j).start()
        for cp in iter_copies(0):
            cp.start()

        cf = c_ref[...].astype(F32)
        sc = jnp.broadcast_to((cf * jax.nn.sigmoid(cf)).astype(BF16), (16, D))

        def mod(j):
            mod_v[j] = _rb(jnp.dot(sc, wm_v[j], preferred_element_type=F32)[0:8])

        def centre(i):
            xf = x_v[_t(i), :].astype(F32)
            mu = jnp.sum(xf, axis=-1, keepdims=True) * (1.0 / D)
            xc = xf - mu
            var = jnp.sum(xc * xc, axis=-1, keepdims=True) * (1.0 / D)
            return xc * lax.rsqrt(var + EPS)

        x_copy(0).wait()
        acc_v[...] = jnp.zeros((S, D), F32)
        xn0 = centre(0)
        cs_v = xn0
        m_copy(0).wait()
        mod(0)
        m_copy(1).wait()
        mod(1)
        wq_copy(0).wait()

        def ln_tile(i, xn):
            h_v[_t(i), :] = (xn * (1.0 + mod_v[1, 0:1, :]) + mod_v[0, 0:1, :]).astype(BF16)

        ln_tile(0, cs_v)
        q_proj(0, 0, 0, 0)
        for i in range(1, NT):
            x_copy(i).wait()
        for cp in first_kv:
            cp.wait()
        for i in range(1, NT):
            ln_tile(i, centre(i))
            q_proj(0, 0, 0, i)
        run_head(' '.join(f'Q{i} X{i} P{i}' for i in range(NT)), 0, 0, 0, 1)
        for j in range(2, 6):
            m_copy(j).wait()
        for j in range(2, 6):
            mod(j)

    pl.run_scoped(prologue, pltpu.VMEM((6, D, D), BF16), pltpu.SemaphoreType.DMA((6,)))

    def rest(wg_v, wu_v, wd_v, r_v, sem_w, sem_out):
        body_seq = 'X0 ' + ' '.join(f'N{i} Q{i} X{i + 1} P{i}' for i in range(NT - 1)) \
            + f' N{NT - 1} Q{NT - 1} P{NT - 1}'

        def body(j, carry):
            for cp in iter_copies(j):
                cp.wait()

            @pl.when(j + 1 < NJ)
            def _():
                for cp in iter_copies(j + 1):
                    cp.start()
            for u in range(G):
                h = G * j + 1 + u
                run_head(body_seq, h, (1 + u) % 2, j * (G // 2) + u // 2 + 1, u % 2)
            return carry

        def w_copies():
            return [pltpu.make_async_copy(wg_hbm, wg_v, sem_w.at[0]),
                    pltpu.make_async_copy(wu_hbm, wu_v, sem_w.at[1]),
                    pltpu.make_async_copy(wd_hbm, wd_v, sem_w.at[2])]

        for cp in last_copies + w_copies():
            cp.start()
        lax.fori_loop(0, NJ, body, 0)
        for cp in last_copies:
            cp.wait()

        ga = mod_v[2, 0:1, :]
        sb = mod_v[3, 0:1, :]
        cb1 = _rb(1.0 + mod_v[4, 0:1, :])
        gb = mod_v[5, 0:1, :]
        wr = wr_ref[...].astype(F32)
        NEG = -jnp.inf
        out_v = h_v

        def out_copy(i):
            return pltpu.make_async_copy(out_v.at[_t(i)], out_hbm.at[0, _t(i)], sem_out.at[i])

        def finish(i):
            att = acc_v[_t(i), :] + out_proj(H - 1, i)
            x1 = _rb(x_v[_t(i), :].astype(F32) + ga * att)
            mu = jnp.sum(x1, axis=-1, keepdims=True) * (1.0 / D)
            xc = x1 - mu
            var = jnp.sum(xc * xc, axis=-1, keepdims=True) * (1.0 / D)
            rs = pltpu.reciprocal(_rb(jnp.sqrt(_rb(_rb(var) + EPS_B))))
            h2 = _rb((x1 - _rb(mu)) * rs * cb1 + sb)
            r = jnp.sum(h2 * wr, axis=-1, keepdims=True)
            x_v[_t(i), :] = x1.astype(BF16)
            for n in range(D // DH):
                k_v[n, _t(i), :] = h2[:, n * DH:(n + 1) * DH].astype(BF16)
            out_v[_t(i), :] = (x1 + gb * h2).astype(BF16)
            r_v[_t(i), :] = jnp.broadcast_to(r, (TQ, 128))

        run_head(' '.join(f'Q{i} N{i} P{i}' for i in range(NT)), H - 1, (H - 1) % 2)
        for i in range(NT):
            finish(i)
        for i in range(NT):
            out_copy(i).start()

        rr = r_v[...]
        rr = jnp.where(rr == rr, rr, NEG)
        ii = lax.broadcasted_iota(jnp.int32, (S, 128), 0)
        m1 = jnp.max(rr, axis=0, keepdims=True)
        i1 = jnp.min(jnp.where(rr == m1, ii, S), axis=0, keepdims=True)
        rr2 = jnp.where(ii == i1, NEG, rr)
        m2 = jnp.max(rr2, axis=0, keepdims=True)
        i2 = jnp.min(jnp.where((rr2 == m2) & (ii != i1), ii, S), axis=0, keepdims=True)
        idx1 = jnp.clip(i1[0, 0], 0, S - 1)
        idx2 = jnp.clip(i2[0, 0], 0, S - 1)
        rid = lax.broadcasted_iota(jnp.int32, (16, D), 0)

        def base_of(idx):
            return pl.multiple_of((idx // 16) * 16, 16)

        def row_of(idx):
            base = base_of(idx)
            pick = lambda blk: jnp.sum(jnp.where(rid == idx - base, blk.astype(F32), 0.0),
                                       axis=0, keepdims=True)
            h2 = jnp.concatenate([k_v[n, pl.ds(base, 16), :] for n in range(D // DH)], axis=1)
            return pick(x_v[pl.ds(base, 16), :]), pick(h2)

        x1a, h2a = row_of(idx1)
        x1b, h2b = row_of(idx2)
        xs = jnp.where(rid == 0, h2a, jnp.where(rid == 1, h2b, 0.0)).astype(BF16)
        for cp in w_copies():
            cp.wait()
        FC = 512
        y = jnp.zeros((16, D), F32)
        for j in range(F // FC):
            cs = slice(j * FC, (j + 1) * FC)
            g = jnp.dot(xs, wg_v[:, cs], preferred_element_type=F32)
            u = jnp.dot(xs, wu_v[:, cs], preferred_element_type=F32)
            a = (g * jax.nn.sigmoid(g) * u).astype(BF16)
            y = y + jnp.dot(a, wd_v[cs, :], preferred_element_type=F32)
        oa = x1a + gb * (h2a + y[0:1] * jax.nn.sigmoid(_rb(m1[:, 0:1])))
        ob = x1b + gb * (h2b + y[1:2] * jax.nn.sigmoid(_rb(m2[:, 0:1])))

        for i in range(NT):
            out_copy(i).wait()

        def patch(idx, row):
            base = base_of(idx)
            blk = out_v[pl.ds(base, 16), :].astype(F32)
            out_v[pl.ds(base, 16), :] = jnp.where(rid == idx - base, row, blk).astype(BF16)
            return base

        def patch_copy(base, k):
            return pltpu.make_async_copy(out_v.at[pl.ds(base, 16)],
                                         out_hbm.at[0, pl.ds(base, 16)], sem_out.at[k])

        b1 = patch(idx1, oa)
        b2 = patch(idx2, ob)
        patch_copy(b1, 0).start()

        @pl.when(b1 != b2)
        def _():
            patch_copy(b2, 1).start()
            patch_copy(b2, 1).wait()
        patch_copy(b1, 0).wait()

    pl.run_scoped(
        rest,
        pltpu.VMEM((D, F), BF16),
        pltpu.VMEM((D, F), BF16),
        pltpu.VMEM((F, D), BF16),
        pltpu.VMEM((S, 128), F32),
        pltpu.SemaphoreType.DMA((3,)),
        pltpu.SemaphoreType.DMA((NT,)),
    )


@jax.jit
def pallas_adaLN_cond__mha_block_cached__moe_arch_mod__prompt_kernel(
    A_x: jax.Array,
    A_k_cache: jax.Array,
    A_v_cache: jax.Array,
    A_wq: jax.Array,
    A_wo: jax.Array,
    B_x: jax.Array,
    B_w_r: jax.Array,
    B_w_gate: jax.Array,
    B_w_up: jax.Array,
    B_w_down: jax.Array,
    c: jax.Array,
    w_mod: jax.Array,
):
    del B_x
    hbm = pl.BlockSpec(memory_space=pl.ANY)
    vmem = pl.BlockSpec(memory_space=pltpu.VMEM)
    return pl.pallas_call(
        _kernel,
        out_shape=jax.ShapeDtypeStruct((1, S, D), BF16),
        in_specs=[vmem, vmem] + [hbm] * 9,
        out_specs=hbm,
        scratch_shapes=[
            pltpu.VMEM((S, D), BF16),
            pltpu.VMEM((S, D), BF16),
            pltpu.VMEM((H, S, DH), BF16),
            pltpu.VMEM((H, S, DH), BF16),
            pltpu.VMEM((H // 2, D, 2 * DH), BF16),
            pltpu.VMEM((H * DH, D), BF16),
            pltpu.VMEM((S, D), F32),
            pltpu.VMEM((S, DH), F32),
            pltpu.VMEM((S, DH), F32),
            pltpu.VMEM((2, S, DH), BF16),
            pltpu.VMEM((6, 8, D), F32),
            pltpu.SemaphoreType.DMA((NT,)),
            pltpu.SemaphoreType.DMA((NJ + 2,)),
            pltpu.SemaphoreType.DMA((NJ + 2,)),
            pltpu.SemaphoreType.DMA((H // 2,)),
            pltpu.SemaphoreType.DMA((H // 2,)),
        ],
        compiler_params=pltpu.CompilerParams(vmem_limit_bytes=127 * 1024 * 1024),
    )(c, B_w_r.reshape(1, D), A_x, A_k_cache, A_v_cache, A_wq, A_wo,
      B_w_gate, B_w_up, B_w_down, w_mod)
```

```python
import jax
import jax.numpy as jnp
import numpy as np
from jax import lax
import jax.experimental.pallas as pl
import jax.experimental.pallas.tpu as pltpu

S, D, H, DH, F = 2048, 1024, 32, 128, 3584
TQ = 256
NT = S // TQ
R_MODE = 1
MC = 256
NG = H // 2
FG = 1
NM = D // MC
URGENT, RELEASE = 21, 0
FS = 512
F32, BF16 = jnp.float32, jnp.bfloat16
QSCALE = float(DH ** -0.5 * np.log2(np.e))
EPS = 1e-5
EPS_B = float(np.asarray(EPS, dtype=np.float32).astype(BF16).astype(np.float32))
NT_DIMS = (((1,), (1,)), ((), ()))

BODY_SEQ = 'Y0 ' + ' '.join(
    f'N{i} ' + f'Q{i} ' + f'Y{i + 1} '
    + f'P{i}' for i in range(NT))
THROTTLE1 = 32
THROTTLE = 32


def _rb(x):
    return x.astype(BF16).astype(F32)


def _recip(x):
    r0 = pltpu.reciprocal(x, approx=True)
    return r0 * (2.0 - x * r0)


def _rowsum(x):
    return jnp.sum(x, axis=-1, keepdims=True)


def _normed(x, ref_rounding=False):
    mu = _rowsum(x) * (1.0 / D)
    var = jnp.maximum(_rowsum(x * x) * (1.0 / D) - mu * mu, 0.0)
    if ref_rounding:
        rs = _recip(_rb(jnp.sqrt(_rb(_rb(var) + EPS_B))))
    else:
        rs = lax.rsqrt(var + EPS)
    return (x - mu) * rs, mu, rs


def _tie(x, ties):
    if not ties:
        return x
    x = jnp.broadcast_to(x, (x.shape[0], DH))
    deps = {k: d for _, k, d in ties}
    return jnp.concatenate(
        [jnp.where(deps[k] * deps[k] < 0.0, 0.0, x[8 * k:8 * k + 8]) if k in deps
         else x[8 * k:8 * k + 8] for k in range(x.shape[0] // 8)], axis=0)


def _dyn(i):
    return pl.ds(pl.multiple_of(i * TQ, TQ), TQ)


def _t(i):
    return slice(i * TQ, (i + 1) * TQ)


def _kernel(c_ref, wr_ref, x_hbm, k_hbm, v_hbm, wq_hbm, wo_hbm, wg_hbm, wu_hbm,
            wd_hbm, wm_hbm, out_hbm,
            x_v, h_v, k_v, v_v, wq_v, wo_v, acc_v, os_v, ls_v, q_v, sc_v, mod_v, wm2_v,
            sem_x, sem_k, sem_v, sem_q, sem_o, sem_m2):

    def x_copy(i):
        r = _dyn(i) if not isinstance(i, int) else _t(i)
        return pltpu.make_async_copy(x_hbm.at[0, r], x_v.at[r], sem_x.at[i])

    def pair(g):
        return pl.ds(pl.multiple_of(g * 2, 2), 2)

    def k_copy(g):
        return pltpu.make_async_copy(k_hbm.at[0, pair(g)], k_v.at[pair(g)], sem_k.at[g])

    def v_copy(g):
        return pltpu.make_async_copy(v_hbm.at[0, pair(g)], v_v.at[pair(g)], sem_v.at[g])

    def wq_copy(g):
        cols = pl.ds(pl.multiple_of(g * 2 * DH, 2 * DH), 2 * DH)
        return pltpu.make_async_copy(wq_hbm.at[:, cols], wq_v.at[g], sem_q.at[g])

    def wo_copy(g):
        src, dst, n = (0, DH, DH) if g == 'first' else (H * DH - DH, H * DH, DH) if g == 'last' \
            else ((2 * g - 1) * DH, 2 * g * DH, 2 * DH)
        al = lambda o: o if isinstance(o, int) else pl.multiple_of(o, DH)
        k = 0 if g == 'first' else NG if g == 'last' else g
        return pltpu.make_async_copy(wo_hbm.at[pl.ds(al(src), n)], wo_v.at[pl.ds(al(dst), n)], sem_o.at[k])

    def m2_copy(j):
        cols = pl.ds(pl.multiple_of(2 * D + j * MC, MC), MC)
        return pltpu.make_async_copy(wm_hbm.at[:, cols], wm2_v.at[j % 2], sem_m2.at[j % 2])

    def q_proj(g, e, i):
        q = jnp.dot(h_v[_t(i), :], wq_v[g, :, e * DH:(e + 1) * DH], preferred_element_type=F32)
        q_v[_t(i), :] = (q * QSCALE).astype(BF16)

    def qk(h, i, ties=()):
        def dot(q, keys):
            return lax.dot_general(q, k_v[h, keys, :], NT_DIMS, preferred_element_type=F32)
        if not ties:
            return dot(q_v[_t(i), :], slice(None))
        q = q_v[_t(i), :].astype(F32)
        return jnp.concatenate(
            [dot(_tie(q, [t for t in ties if t[0] <= r]).astype(BF16), slice(r * 512, (r + 1) * 512))
             for r in range(4)], axis=1)

    def pv(h, s, ties=()):
        m = jnp.max(s, axis=-1, keepdims=True)
        if ties:
            m = jnp.concatenate(
                [jnp.concatenate([_tie(m, [t for t in ties if t[0] <= r])] * 4, axis=1)
                 for r in range(4)], axis=1)
        p = jnp.exp2(s - m)
        l = p[:, 0:128]
        for j in range(1, S // 128):
            l = l + p[:, j * 128:(j + 1) * 128]
        return jnp.dot(p.astype(BF16), v_v[h], preferred_element_type=F32), l

    def out_proj(h, o, l, ties=(), w=None):
        inv = _tie(_recip(_rowsum(l)), ties)
        if w is None:
            w = wo_v[pl.ds(pl.multiple_of((h + 1) * DH, DH), DH), :]
        return jnp.dot((o * inv).astype(BF16), w, preferred_element_type=F32)

    def mod_part(j, e):
        cs = slice(e * DH, (e + 1) * DH)
        mod_v[j, :, cs] = jnp.dot(sc_v[...], wm2_v[j % 2, :, cs], preferred_element_type=F32)[0:8]

    def run_head(g, e):
        h = 2 * g + e
        for tok in BODY_SEQ.split():
            kind, i = tok[0], int(tok[1:])
            if kind == 'Q':
                s = qk(h, i)
            elif kind == 'P':
                os_v[_t(i), :], ls_v[_t(i), :] = pv(h, s)
            elif kind == 'N':
                acc_v[_t(i), :] += out_proj(h - 1, os_v[_t(i), :], ls_v[_t(i), :])
            elif kind == 'Y' and i < NT:
                q_proj(g, e, i)
            else:
                mod_part(g, e)

    def prologue(wm_v, h1_v, sem_m):
        def m_copy(j):
            r = slice(j * DH, (j + 1) * DH)
            return pltpu.make_async_copy(wm_hbm.at[r, 0:2 * D], wm_v.at[r], sem_m.at[j])

        nk = D // DH
        urgent = ([m_copy(j) for j in range(nk)] + [x_copy(i) for i in range(NT)]
                  + [wq_copy(0), wo_copy('first'), m2_copy(0), k_copy(0), v_copy(0)])
        for cp in urgent[:URGENT]:
            cp.start()

        cf = c_ref[...].astype(F32)
        sc = jnp.broadcast_to((cf * jax.nn.sigmoid(cf)).astype(BF16), (16, D))
        sc_v[...] = sc

        @pl.loop(0, NT)
        def _(i):
            acc_v[_dyn(i), :] = jnp.zeros((TQ, D), F32)


        os_v[...] = jnp.zeros((S, DH), F32)
        ls_v[...] = jnp.ones((S, DH), F32)
        wo_v[0:DH, :] = jnp.zeros((DH, D), BF16)
        y = 0.0
        for j in range(nk):
            m_copy(j).wait()
            if j == RELEASE:
                for cp in urgent[URGENT:]:
                    cp.start()
            y = y + jnp.dot(sc[:, j * DH:(j + 1) * DH], wm_v[j * DH:(j + 1) * DH, :],
                            preferred_element_type=F32)[0:8]
        h1_v[0] = _rb(y[:, :D])
        h1_v[1] = 1.0 + _rb(y[:, D:])

        def ln_tile(i, carry):
            x_copy(i).wait()
            x = x_v[_dyn(i), :].astype(F32)
            _, mu, rs = _normed(x)
            rs, c1, c0 = jnp.broadcast_to(rs, (TQ, DH)), h1_v[1, 0:1, :], h1_v[0, 0:1, :]
            outs = []
            for e in range(TQ // 8):
                g = slice(8 * e, 8 * e + 8)
                re = rs[g]
                if e >= THROTTLE1:
                    d = outs[e - THROTTLE1][:, D - DH:]
                    re = jnp.where(d * d < 0.0, 0.0, re)
                outs.append((x[g] - mu[g]) * jnp.concatenate([re] * (D // DH), axis=1) * c1 + c0)
            h_v[_dyn(i), :] = jnp.concatenate(outs, axis=0).astype(BF16)
            return carry

        lax.fori_loop(0, NT, ln_tile, 0)

    pl.run_scoped(prologue, pltpu.VMEM((D, 2 * D), BF16), pltpu.VMEM((2, 8, D), F32),
                  pltpu.SemaphoreType.DMA((2 * NM,)))

    def rest(wg_v, wu_v, wd_v, st_v, sem_w, sem_out):
        def w_copies(j):
            c = pl.ds(pl.multiple_of(j * FS, FS), FS)
            return [pltpu.make_async_copy(wg_hbm.at[:, c], wg_v.at[j], sem_w.at[0, j]),
                    pltpu.make_async_copy(wu_hbm.at[:, c], wu_v.at[j], sem_w.at[1, j]),
                    pltpu.make_async_copy(wd_hbm.at[c], wd_v.at[c], sem_w.at[2, j])]

        def body(g, carry):
            for cp in (k_copy(g), v_copy(g), wq_copy(g), m2_copy(g)):
                cp.wait()

            @pl.when(g == 0)
            def _():
                wo_copy('first').wait()

            @pl.when(g > 0)
            def _():
                wo_copy(g).wait()

            @pl.when(g + 1 < NG)
            def _():
                for cp in (k_copy(g + 1), v_copy(g + 1), wq_copy(g + 1), wo_copy(g + 1), m2_copy(g + 1)):
                    cp.start()

            @pl.when(g < F // FS)
            def _():
                for cp in w_copies(g):
                    cp.start()
            run_head(g, 0)
            run_head(g, 1)
            return carry

        wo_copy('last').start()
        lax.fori_loop(0, NG, body, 0)
        wo_copy('last').wait()

        def vec(n):
            return _rb(jnp.concatenate([mod_v[n * NM + j, 0:1, :] for j in range(NM)], axis=1))

        ga, sb, gb = vec(0), vec(1), vec(3)
        cb1 = _rb(1.0 + vec(2))
        wr = wr_ref[...].astype(F32)
        wc = cb1 * wr
        wc_sum, sw_sum = _rowsum(wc), _rowsum(sb * wr)
        NEG = -jnp.inf
        out_v = h_v

        def out_copy(n):
            r = pl.ds(pl.multiple_of(n * FG * TQ, FG * TQ), FG * TQ)
            return pltpu.make_async_copy(out_v.at[r], out_hbm.at[0, r], sem_out.at[n])

        gc, gs = gb * cb1, gb * sb

        def rows(i):
            return pl.ds(pl.multiple_of(i * TQ, TQ), TQ)

        def finish(i, top):
            y = out_proj(H - 1, os_v[rows(i), :], ls_v[rows(i), :])
            x1b = (x_v[rows(i), :].astype(F32) + ga * (acc_v[rows(i), :] + y)).astype(BF16)
            x_v[rows(i), :] = x1b
            x1 = x1b.astype(F32)
            xn, mu, rs = _normed(x1, True)
            st_v[0, rows(i), :] = jnp.broadcast_to(mu, (TQ, DH))
            st_v[1, rows(i), :] = jnp.broadcast_to(rs, (TQ, DH))
            outs, rs_, done, rs_full = [], [], [], jnp.broadcast_to(rs, (TQ, DH))
            for e in range(TQ // 8):
                g = slice(8 * e, 8 * e + 8)
                re = rs_full[g]
                if e >= THROTTLE:
                    re = jnp.where(done[e - THROTTLE] < 0.0, 0.0, re)
                xg = (x1[g] - mu[g]) * jnp.concatenate([re] * (D // DH), axis=1)
                if R_MODE == 0:
                    o = x1[g] + (xg * gc + gs)
                    rg = re * (_rowsum(x1[g] * wc) - mu[g] * wc_sum) + sw_sum
                else:
                    h2 = xg * cb1 + sb
                    o = x1[g] + gb * h2
                    rg = _rowsum(h2 * wr)
                if R_MODE == 0:
                    d = o[:, D - DH:]
                else:
                    d = rg
                outs.append(o), rs_.append(rg), done.append(d * d)
            out_v[rows(i), :] = jnp.concatenate(outs, axis=0).astype(BF16)
            m1, m2, k1, k2 = top
            for e in range(TQ // 8):
                re, ke = rs_[e][:, 0:1], i * (TQ // 8) + e
                g1, g2 = re > m1, re > m2
                m2 = jnp.where(g1, m1, jnp.where(g2, re, m2))
                k2 = jnp.where(g1, k1, jnp.where(g2, ke, k2))
                m1 = jnp.where(g1, re, m1)
                k1 = jnp.where(g1, ke, k1)
            return m1, m2, k1, k2

        def finish_group(n, top):
            for e in range(FG):
                top = finish(n * FG + e, top)
            out_copy(n).start()
            return top

        top = lax.fori_loop(0, NT // FG, finish_group, (
            jnp.full((8, 1), NEG, F32), jnp.full((8, 1), NEG, F32),
            jnp.zeros((8, 1), jnp.int32), jnp.ones((8, 1), jnp.int32)))

        m1, m2, k1, k2 = top
        sub = lax.broadcasted_iota(jnp.int32, (8, 1), 0)
        i1, i2 = k1 * 8 + sub, k2 * 8 + sub
        b1 = jnp.max(m1, axis=0, keepdims=True)
        j1 = jnp.min(jnp.where(m1 == b1, i1, S), axis=0, keepdims=True)
        won = i1 == j1
        n1 = jnp.where(won, m2, m1)
        ni = jnp.where(won, i2, i1)
        b2 = jnp.max(n1, axis=0, keepdims=True)
        j2 = jnp.min(jnp.where((n1 == b2) & (ni != j1), ni, S), axis=0, keepdims=True)
        idx1 = jnp.clip(j1[0, 0], 0, S - 1)
        idx2 = jnp.clip(j2[0, 0], 0, S - 1)
        rid = lax.broadcasted_iota(jnp.int32, (16, D), 0)

        def base_of(idx):
            return pl.multiple_of((idx // 16) * 16, 16)

        def h2_row(idx):
            base = base_of(idx)
            blk = x_v[pl.ds(base, 16), :].astype(F32)
            x1 = jnp.sum(jnp.where(rid == idx - base, blk, 0.0), axis=0, keepdims=True)
            mu, rs = st_v[0, pl.ds(idx, 1), :][:, 0:1], st_v[1, pl.ds(idx, 1), :][:, 0:1]
            return (x1 - mu) * rs * cb1 + sb

        h2a, h2b = h2_row(idx1), h2_row(idx2)
        xs = jnp.where(rid == 0, h2a, jnp.where(rid == 1, h2b, 0.0)).astype(BF16)
        for j in range(F // FS):
            for cp in w_copies(j):
                cp.wait()
        FC = FS
        acts = []
        for j in range(F // FC):
            cs = slice(j * FC, (j + 1) * FC)
            g = jnp.dot(xs, wg_v[j], preferred_element_type=F32)
            u = jnp.dot(xs, wu_v[j], preferred_element_type=F32)
            acts.append((g * jax.nn.sigmoid(g) * u).astype(BF16))
        y = None
        for j, a in enumerate(acts):
            yj = jnp.dot(a, wd_v[j * FC:(j + 1) * FC, :], preferred_element_type=F32)
            y = yj if y is None else y + yj
        ua = gb * (y[0:1] * jax.nn.sigmoid(_rb(b1)))
        ub = gb * (y[1:2] * jax.nn.sigmoid(_rb(b2)))

        for n in range(NT // FG):
            out_copy(n).wait()

        def patch(idx, row):
            base = base_of(idx)
            blk = out_v[pl.ds(base, 16), :].astype(F32)
            out_v[pl.ds(base, 16), :] = jnp.where(rid == idx - base, blk + row, blk).astype(BF16)
            return base

        def patch_copy(base, k):
            return pltpu.make_async_copy(out_v.at[pl.ds(base, 16)],
                                         out_hbm.at[0, pl.ds(base, 16)], sem_out.at[k])

        p1 = patch(idx1, ua)
        p2 = patch(idx2, ub)
        patch_copy(p1, 0).start()

        @pl.when(p1 != p2)
        def _():
            patch_copy(p2, 1).start()
            patch_copy(p2, 1).wait()
        patch_copy(p1, 0).wait()

    pl.run_scoped(
        rest,
        pltpu.VMEM((F // FS, D, FS), BF16),
        pltpu.VMEM((F // FS, D, FS), BF16),
        pltpu.VMEM((F, D), BF16),
        pltpu.VMEM((2, S, DH), F32),
        pltpu.SemaphoreType.DMA((3, F // FS)),
        pltpu.SemaphoreType.DMA((NT,)),
    )


@jax.jit
def pallas_adaLN_cond__mha_block_cached__moe_arch_mod__prompt_kernel(
    A_x: jax.Array,
    A_k_cache: jax.Array,
    A_v_cache: jax.Array,
    A_wq: jax.Array,
    A_wo: jax.Array,
    B_x: jax.Array,
    B_w_r: jax.Array,
    B_w_gate: jax.Array,
    B_w_up: jax.Array,
    B_w_down: jax.Array,
    c: jax.Array,
    w_mod: jax.Array,
):
    del B_x
    hbm = pl.BlockSpec(memory_space=pl.ANY)
    vmem = pl.BlockSpec(memory_space=pltpu.VMEM)
    return pl.pallas_call(
        _kernel,
        out_shape=jax.ShapeDtypeStruct((1, S, D), BF16),
        in_specs=[vmem, vmem] + [hbm] * 9,
        out_specs=hbm,
        scratch_shapes=[
            pltpu.VMEM((S, D), BF16),
            pltpu.VMEM((S, D), BF16),
            pltpu.VMEM((H, S, DH), BF16),
            pltpu.VMEM((H, S, DH), BF16),
            pltpu.VMEM((NG, D, 2 * DH), BF16),
            pltpu.VMEM((H * DH + DH, D), BF16),
            pltpu.VMEM((S, D), F32),
            pltpu.VMEM((S, DH), F32),
            pltpu.VMEM((S, DH), F32),
            pltpu.VMEM((S, DH), BF16),
            pltpu.VMEM((16, D), BF16),
            pltpu.VMEM((4 * NM, 8, MC), F32),
            pltpu.VMEM((2, D, MC), BF16),
            pltpu.SemaphoreType.DMA((NT,)),
            pltpu.SemaphoreType.DMA((NG,)),
            pltpu.SemaphoreType.DMA((NG,)),
            pltpu.SemaphoreType.DMA((NG,)),
            pltpu.SemaphoreType.DMA((NG + 1,)),
            pltpu.SemaphoreType.DMA((2,)),
        ],
        compiler_params=pltpu.CompilerParams(vmem_limit_bytes=127 * 1024 * 1024),
    )(c, B_w_r.reshape(1, D), A_x, A_k_cache, A_v_cache, A_wq, A_wo,
      B_w_gate, B_w_up, B_w_down, w_mod)
```

```python
import jax
import jax.numpy as jnp
import numpy as np
from jax import lax
import jax.experimental.pallas as pl
import jax.experimental.pallas.tpu as pltpu

S, D, H, DH, F = 2048, 1024, 32, 128, 3584
TQ = 256
NT = S // TQ
R_MODE = 1
MC = 256
NG = H // 2
FG = 1
NM = D // MC
URGENT, RELEASE = 21, 0
FS = 512
F32, BF16 = jnp.float32, jnp.bfloat16
QSCALE = float(DH ** -0.5 * np.log2(np.e))
EPS = 1e-5
EPS_B = float(np.asarray(EPS, dtype=np.float32).astype(BF16).astype(np.float32))
NT_DIMS = (((1,), (1,)), ((), ()))

BODY_SEQ = 'Y0 ' + ' '.join(
    f'N{i} ' + f'Q{i} ' + f'Y{i + 1} '
    + f'P{i}' for i in range(NT))
THROTTLE1 = 32
THROTTLE = 32


def _rb(x):
    return x.astype(BF16).astype(F32)


def _recip(x):
    r0 = pltpu.reciprocal(x, approx=True)
    return r0 * (2.0 - x * r0)


def _rowsum(x):
    return jnp.sum(x, axis=-1, keepdims=True)


def _normed(x, ref_rounding=False):
    mu = _rowsum(x) * (1.0 / D)
    var = jnp.maximum(_rowsum(x * x) * (1.0 / D) - mu * mu, 0.0)
    if ref_rounding:
        rs = _recip(_rb(jnp.sqrt(_rb(_rb(var) + EPS_B))))
    else:
        rs = lax.rsqrt(var + EPS)
    return (x - mu) * rs, mu, rs


def _tie(x, ties):
    if not ties:
        return x
    x = jnp.broadcast_to(x, (x.shape[0], DH))
    deps = {k: d for _, k, d in ties}
    return jnp.concatenate(
        [jnp.where(deps[k] * deps[k] < 0.0, 0.0, x[8 * k:8 * k + 8]) if k in deps
         else x[8 * k:8 * k + 8] for k in range(x.shape[0] // 8)], axis=0)


def _dyn(i):
    return pl.ds(pl.multiple_of(i * TQ, TQ), TQ)


def _t(i):
    return slice(i * TQ, (i + 1) * TQ)


def _kernel(c_ref, wr_ref, x_hbm, k_hbm, v_hbm, wq_hbm, wo_hbm, wg_hbm, wu_hbm,
            wd_hbm, wm_hbm, out_hbm,
            x_v, h_v, k_v, v_v, wq_v, wo_v, acc_v, os_v, ls_v, q_v, sc_v, mod_v, wm2_v,
            sem_x, sem_k, sem_v, sem_q, sem_o, sem_m2):

    def x_copy(i):
        r = _dyn(i) if not isinstance(i, int) else _t(i)
        return pltpu.make_async_copy(x_hbm.at[0, r], x_v.at[r], sem_x.at[i])

    def pair(g):
        return pl.ds(pl.multiple_of(g * 2, 2), 2)

    def k_copy(g):
        return pltpu.make_async_copy(k_hbm.at[0, pair(g)], k_v.at[pair(g)], sem_k.at[g])

    def v_copy(g):
        return pltpu.make_async_copy(v_hbm.at[0, pair(g)], v_v.at[pair(g)], sem_v.at[g])

    def wq_copy(g):
        cols = pl.ds(pl.multiple_of(g * 2 * DH, 2 * DH), 2 * DH)
        return pltpu.make_async_copy(wq_hbm.at[:, cols], wq_v.at[g], sem_q.at[g])

    def wo_copy(g):
        src, dst, n = (0, DH, DH) if g == 'first' else (H * DH - DH, H * DH, DH) if g == 'last' \
            else ((2 * g - 1) * DH, 2 * g * DH, 2 * DH)
        al = lambda o: o if isinstance(o, int) else pl.multiple_of(o, DH)
        k = 0 if g == 'first' else NG if g == 'last' else g
        return pltpu.make_async_copy(wo_hbm.at[pl.ds(al(src), n)], wo_v.at[pl.ds(al(dst), n)], sem_o.at[k])

    def m2_copy(j):
        cols = pl.ds(pl.multiple_of(2 * D + j * MC, MC), MC)
        return pltpu.make_async_copy(wm_hbm.at[:, cols], wm2_v.at[j % 2], sem_m2.at[j % 2])

    def q_proj(g, e, i):
        q = jnp.dot(h_v[_t(i), :], wq_v[g, :, e * DH:(e + 1) * DH], preferred_element_type=F32)
        q_v[_t(i), :] = (q * QSCALE).astype(BF16)

    def qk(h, i, ties=()):
        def dot(q, keys):
            return lax.dot_general(q, k_v[h, keys, :], NT_DIMS, preferred_element_type=F32)
        if not ties:
            return dot(q_v[_t(i), :], slice(None))
        q = q_v[_t(i), :].astype(F32)
        return jnp.concatenate(
            [dot(_tie(q, [t for t in ties if t[0] <= r]).astype(BF16), slice(r * 512, (r + 1) * 512))
             for r in range(4)], axis=1)

    def pv(h, s, ties=()):
        m = jnp.max(s, axis=-1, keepdims=True)
        if ties:
            m = jnp.concatenate(
                [jnp.concatenate([_tie(m, [t for t in ties if t[0] <= r])] * 4, axis=1)
                 for r in range(4)], axis=1)
        p = jnp.exp2(s - m)
        l = p[:, 0:128]
        for j in range(1, S // 128):
            l = l + p[:, j * 128:(j + 1) * 128]
        return jnp.dot(p.astype(BF16), v_v[h], preferred_element_type=F32), l

    def out_proj(h, o, l, ties=(), w=None):
        inv = _tie(_recip(_rowsum(l)), ties)
        if w is None:
            w = wo_v[pl.ds(pl.multiple_of((h + 1) * DH, DH), DH), :]
        return jnp.dot((o * inv).astype(BF16), w, preferred_element_type=F32)

    def mod_part(j, e):
        cs = slice(e * DH, (e + 1) * DH)
        mod_v[j, :, cs] = jnp.dot(sc_v[...], wm2_v[j % 2, :, cs], preferred_element_type=F32)[0:8]

    def run_head(g, e):
        h = 2 * g + e
        for tok in BODY_SEQ.split():
            kind, i = tok[0], int(tok[1:])
            if kind == 'Q':
                s = qk(h, i)
            elif kind == 'P':
                os_v[_t(i), :], ls_v[_t(i), :] = pv(h, s)
            elif kind == 'N':
                acc_v[_t(i), :] += out_proj(h - 1, os_v[_t(i), :], ls_v[_t(i), :])
            elif kind == 'Y' and i < NT:
                q_proj(g, e, i)
            else:
                mod_part(g, e)

    def prologue(wm_v, h1_v, sem_m):
        def m_copy(j):
            r = slice(j * DH, (j + 1) * DH)
            return pltpu.make_async_copy(wm_hbm.at[r, 0:2 * D], wm_v.at[r], sem_m.at[j])

        nk = D // DH
        urgent = ([x_copy(i) for i in range(NT)] + [m_copy(j) for j in range(nk)]
                  + [wq_copy(0), wo_copy('first'), m2_copy(0), k_copy(0), v_copy(0)])
        for cp in urgent[:URGENT]:
            cp.start()

        cf = c_ref[...].astype(F32)
        sc = jnp.broadcast_to((cf * jax.nn.sigmoid(cf)).astype(BF16), (16, D))
        sc_v[...] = sc

        @pl.loop(0, NT)
        def _(i):
            x_copy(i).wait()
            acc_v[_dyn(i), :] = _normed(x_v[_dyn(i), :].astype(F32))[0]

        os_v[...] = jnp.zeros((S, DH), F32)
        ls_v[...] = jnp.ones((S, DH), F32)
        wo_v[0:DH, :] = jnp.zeros((DH, D), BF16)
        y = 0.0
        for j in range(nk):
            m_copy(j).wait()
            if j == RELEASE:
                for cp in urgent[URGENT:]:
                    cp.start()
            y = y + jnp.dot(sc[:, j * DH:(j + 1) * DH], wm_v[j * DH:(j + 1) * DH, :],
                            preferred_element_type=F32)[0:8]
        h1_v[0] = _rb(y[:, :D])
        h1_v[1] = 1.0 + _rb(y[:, D:])

        @pl.loop(0, NT)
        def _(i):
            h_v[_dyn(i), :] = (acc_v[_dyn(i), :] * h1_v[1, 0:1, :] + h1_v[0, 0:1, :]).astype(BF16)
            acc_v[_dyn(i), :] = jnp.zeros((TQ, D), F32)

    pl.run_scoped(prologue, pltpu.VMEM((D, 2 * D), BF16), pltpu.VMEM((2, 8, D), F32),
                  pltpu.SemaphoreType.DMA((2 * NM,)))

    def rest(wg_v, wu_v, wd_v, st_v, sem_w, sem_out):
        def w_copies(j):
            c = pl.ds(pl.multiple_of(j * FS, FS), FS)
            return [pltpu.make_async_copy(wg_hbm.at[:, c], wg_v.at[j], sem_w.at[0, j]),
                    pltpu.make_async_copy(wu_hbm.at[:, c], wu_v.at[j], sem_w.at[1, j]),
                    pltpu.make_async_copy(wd_hbm.at[c], wd_v.at[c], sem_w.at[2, j])]

        def body(g, carry):
            for cp in (k_copy(g), v_copy(g), wq_copy(g), m2_copy(g)):
                cp.wait()

            @pl.when(g == 0)
            def _():
                wo_copy('first').wait()

            @pl.when(g > 0)
            def _():
                wo_copy(g).wait()

            @pl.when(g + 1 < NG)
            def _():
                for cp in (k_copy(g + 1), v_copy(g + 1), wq_copy(g + 1), wo_copy(g + 1), m2_copy(g + 1)):
                    cp.start()

            @pl.when(g < F // FS)
            def _():
                for cp in w_copies(g):
                    cp.start()
            run_head(g, 0)
            run_head(g, 1)
            return carry

        wo_copy('last').start()
        lax.fori_loop(0, NG, body, 0)
        wo_copy('last').wait()

        def vec(n):
            return _rb(jnp.concatenate([mod_v[n * NM + j, 0:1, :] for j in range(NM)], axis=1))

        ga, sb, gb = vec(0), vec(1), vec(3)
        cb1 = _rb(1.0 + vec(2))
        wr = wr_ref[...].astype(F32).reshape(1, D)
        wc = cb1 * wr
        wc_sum, sw_sum = _rowsum(wc), _rowsum(sb * wr)
        NEG = -jnp.inf
        out_v = h_v

        def out_copy(n):
            r = pl.ds(pl.multiple_of(n * FG * TQ, FG * TQ), FG * TQ)
            return pltpu.make_async_copy(out_v.at[r], out_hbm.at[0, r], sem_out.at[n])

        gc, gs = gb * cb1, gb * sb

        def rows(i):
            return pl.ds(pl.multiple_of(i * TQ, TQ), TQ)

        def finish(i, top):
            y = out_proj(H - 1, os_v[rows(i), :], ls_v[rows(i), :])
            x1b = (x_v[rows(i), :].astype(F32) + ga * (acc_v[rows(i), :] + y)).astype(BF16)
            x_v[rows(i), :] = x1b
            x1 = x1b.astype(F32)
            xn, mu, rs = _normed(x1, True)
            st_v[0, rows(i), :] = jnp.broadcast_to(mu, (TQ, DH))
            st_v[1, rows(i), :] = jnp.broadcast_to(rs, (TQ, DH))
            outs, rs_, done, rs_full = [], [], [], jnp.broadcast_to(rs, (TQ, DH))
            for e in range(TQ // 8):
                g = slice(8 * e, 8 * e + 8)
                re = rs_full[g]
                if e >= THROTTLE:
                    re = jnp.where(done[e - THROTTLE] < 0.0, 0.0, re)
                xg = (x1[g] - mu[g]) * jnp.concatenate([re] * (D // DH), axis=1)
                if R_MODE == 0:
                    o = x1[g] + (xg * gc + gs)
                    rg = re * (_rowsum(x1[g] * wc) - mu[g] * wc_sum) + sw_sum
                else:
                    h2 = xg * cb1 + sb
                    o = x1[g] + gb * h2
                    rg = _rowsum(h2 * wr)
                if R_MODE == 0:
                    d = o[:, D - DH:]
                else:
                    d = rg
                outs.append(o), rs_.append(rg), done.append(d * d)
            out_v[rows(i), :] = jnp.concatenate(outs, axis=0).astype(BF16)
            m1, m2, k1, k2 = top
            for e in range(TQ // 8):
                re, ke = rs_[e][:, 0:1], i * (TQ // 8) + e
                g1, g2 = re > m1, re > m2
                m2 = jnp.where(g1, m1, jnp.where(g2, re, m2))
                k2 = jnp.where(g1, k1, jnp.where(g2, ke, k2))
                m1 = jnp.where(g1, re, m1)
                k1 = jnp.where(g1, ke, k1)
            return m1, m2, k1, k2

        def finish_group(n, top):
            for e in range(FG):
                top = finish(n * FG + e, top)
            out_copy(n).start()
            return top

        top = lax.fori_loop(0, NT // FG, finish_group, (
            jnp.full((8, 1), NEG, F32), jnp.full((8, 1), NEG, F32),
            jnp.zeros((8, 1), jnp.int32), jnp.ones((8, 1), jnp.int32)))

        m1, m2, k1, k2 = top
        sub = lax.broadcasted_iota(jnp.int32, (8, 1), 0)
        i1, i2 = k1 * 8 + sub, k2 * 8 + sub
        b1 = jnp.max(m1, axis=0, keepdims=True)
        j1 = jnp.min(jnp.where(m1 == b1, i1, S), axis=0, keepdims=True)
        won = i1 == j1
        n1 = jnp.where(won, m2, m1)
        ni = jnp.where(won, i2, i1)
        b2 = jnp.max(n1, axis=0, keepdims=True)
        j2 = jnp.min(jnp.where((n1 == b2) & (ni != j1), ni, S), axis=0, keepdims=True)
        idx1 = jnp.clip(j1[0, 0], 0, S - 1)
        idx2 = jnp.clip(j2[0, 0], 0, S - 1)
        rid = lax.broadcasted_iota(jnp.int32, (16, D), 0)

        def base_of(idx):
            return pl.multiple_of((idx // 16) * 16, 16)

        def h2_row(idx):
            base = base_of(idx)
            blk = x_v[pl.ds(base, 16), :].astype(F32)
            x1 = jnp.sum(jnp.where(rid == idx - base, blk, 0.0), axis=0, keepdims=True)
            mu, rs = st_v[0, pl.ds(idx, 1), :][:, 0:1], st_v[1, pl.ds(idx, 1), :][:, 0:1]
            return (x1 - mu) * rs * cb1 + sb

        h2a, h2b = h2_row(idx1), h2_row(idx2)
        xs = jnp.where(rid == 0, h2a, jnp.where(rid == 1, h2b, 0.0)).astype(BF16)
        for j in range(F // FS):
            for cp in w_copies(j):
                cp.wait()
        FC = FS
        acts = []
        for j in range(F // FC):
            cs = slice(j * FC, (j + 1) * FC)
            g = jnp.dot(xs, wg_v[j], preferred_element_type=F32)
            u = jnp.dot(xs, wu_v[j], preferred_element_type=F32)
            acts.append((g * jax.nn.sigmoid(g) * u).astype(BF16))
        y = None
        for j, a in enumerate(acts):
            yj = jnp.dot(a, wd_v[j * FC:(j + 1) * FC, :], preferred_element_type=F32)
            y = yj if y is None else y + yj
        ua = gb * (y[0:1] * jax.nn.sigmoid(_rb(b1)))
        ub = gb * (y[1:2] * jax.nn.sigmoid(_rb(b2)))

        for n in range(NT // FG):
            out_copy(n).wait()

        def patch(idx, row):
            base = base_of(idx)
            blk = out_v[pl.ds(base, 16), :].astype(F32)
            out_v[pl.ds(base, 16), :] = jnp.where(rid == idx - base, blk + row, blk).astype(BF16)
            return base

        def patch_copy(base, k):
            return pltpu.make_async_copy(out_v.at[pl.ds(base, 16)],
                                         out_hbm.at[0, pl.ds(base, 16)], sem_out.at[k])

        p1 = patch(idx1, ua)
        p2 = patch(idx2, ub)
        patch_copy(p1, 0).start()

        @pl.when(p1 != p2)
        def _():
            patch_copy(p2, 1).start()
            patch_copy(p2, 1).wait()
        patch_copy(p1, 0).wait()

    pl.run_scoped(
        rest,
        pltpu.VMEM((F // FS, D, FS), BF16),
        pltpu.VMEM((F // FS, D, FS), BF16),
        pltpu.VMEM((F, D), BF16),
        pltpu.VMEM((2, S, DH), F32),
        pltpu.SemaphoreType.DMA((3, F // FS)),
        pltpu.SemaphoreType.DMA((NT,)),
    )


@jax.jit
def pallas_adaLN_cond__mha_block_cached__moe_arch_mod__prompt_kernel(
    A_x: jax.Array,
    A_k_cache: jax.Array,
    A_v_cache: jax.Array,
    A_wq: jax.Array,
    A_wo: jax.Array,
    B_x: jax.Array,
    B_w_r: jax.Array,
    B_w_gate: jax.Array,
    B_w_up: jax.Array,
    B_w_down: jax.Array,
    c: jax.Array,
    w_mod: jax.Array,
):
    del B_x
    hbm = pl.BlockSpec(memory_space=pl.ANY)
    vmem = pl.BlockSpec(memory_space=pltpu.VMEM)
    return pl.pallas_call(
        _kernel,
        out_shape=jax.ShapeDtypeStruct((1, S, D), BF16),
        in_specs=[vmem, vmem] + [hbm] * 9,
        out_specs=hbm,
        scratch_shapes=[
            pltpu.VMEM((S, D), BF16),
            pltpu.VMEM((S, D), BF16),
            pltpu.VMEM((H, S, DH), BF16),
            pltpu.VMEM((H, S, DH), BF16),
            pltpu.VMEM((NG, D, 2 * DH), BF16),
            pltpu.VMEM((H * DH + DH, D), BF16),
            pltpu.VMEM((S, D), F32),
            pltpu.VMEM((S, DH), F32),
            pltpu.VMEM((S, DH), F32),
            pltpu.VMEM((S, DH), BF16),
            pltpu.VMEM((16, D), BF16),
            pltpu.VMEM((4 * NM, 8, MC), F32),
            pltpu.VMEM((2, D, MC), BF16),
            pltpu.SemaphoreType.DMA((NT,)),
            pltpu.SemaphoreType.DMA((NG,)),
            pltpu.SemaphoreType.DMA((NG,)),
            pltpu.SemaphoreType.DMA((NG,)),
            pltpu.SemaphoreType.DMA((NG + 1,)),
            pltpu.SemaphoreType.DMA((2,)),
        ],
        compiler_params=pltpu.CompilerParams(vmem_limit_bytes=127 * 1024 * 1024),
    )(c, B_w_r, A_x, A_k_cache, A_v_cache, A_wq, A_wo,
      B_w_gate, B_w_up, B_w_down, w_mod)
```

```python
import jax
import jax.numpy as jnp
import numpy as np
from jax import lax
import jax.experimental.pallas as pl
import jax.experimental.pallas.tpu as pltpu

S, D, H, DH, F = 2048, 1024, 32, 128, 3584
TQ = 256
NT = S // TQ
R_MODE = 0
MC = 256
NG = H // 2
FG = 2
NM = D // MC
URGENT, RELEASE = 21, 0
FS = 512
F32, BF16 = jnp.float32, jnp.bfloat16
QSCALE = float(DH ** -0.5 * np.log2(np.e))
EPS = 1e-5
EPS_B = float(np.asarray(EPS, dtype=np.float32).astype(BF16).astype(np.float32))
NT_DIMS = (((1,), (1,)), ((), ()))

BODY_SEQ = 'Y0 ' + ' '.join(
    f'N{i} ' + f'Q{i} ' + f'Y{i + 1} '
    + f'P{i}' for i in range(NT))
THROTTLE1 = 32
THROTTLE = 6


def _rb(x):
    return x.astype(BF16).astype(F32)


def _recip(x):
    r0 = pltpu.reciprocal(x, approx=True)
    return r0 * (2.0 - x * r0)


def _rowsum(x):
    return jnp.sum(x, axis=-1, keepdims=True)


def _normed(x, ref_rounding=False):
    mu = _rowsum(x) * (1.0 / D)
    var = jnp.maximum(_rowsum(x * x) * (1.0 / D) - mu * mu, 0.0)
    if ref_rounding:
        v = _rb(_rb(var) + EPS_B)
        rs = _recip(_rb(v * lax.rsqrt(v)))
    else:
        rs = lax.rsqrt(var + EPS)
    return (x - mu) * rs, mu, rs


def _tie(x, ties):
    if not ties:
        return x
    x = jnp.broadcast_to(x, (x.shape[0], DH))
    deps = {k: d for _, k, d in ties}
    return jnp.concatenate(
        [jnp.where(deps[k] * deps[k] < 0.0, 0.0, x[8 * k:8 * k + 8]) if k in deps
         else x[8 * k:8 * k + 8] for k in range(x.shape[0] // 8)], axis=0)


def _dyn(i):
    return pl.ds(pl.multiple_of(i * TQ, TQ), TQ)


def _t(i):
    return slice(i * TQ, (i + 1) * TQ)


def _kernel(c_ref, wr_ref, x_hbm, k_hbm, v_hbm, wq_hbm, wo_hbm, wg_hbm, wu_hbm,
            wd_hbm, wm_hbm, out_hbm,
            x_v, h_v, k_v, v_v, wq_v, wo_v, acc_v, os_v, ls_v, q_v, sc_v, mod_v, wm2_v,
            sem_x, sem_k, sem_v, sem_q, sem_o, sem_m2):

    def x_copy(i):
        r = _dyn(i) if not isinstance(i, int) else _t(i)
        return pltpu.make_async_copy(x_hbm.at[0, r], x_v.at[r], sem_x.at[i])

    def pair(g):
        return pl.ds(pl.multiple_of(g * 2, 2), 2)

    def k_copy(g):
        return pltpu.make_async_copy(k_hbm.at[0, pair(g)], k_v.at[pair(g)], sem_k.at[g])

    def v_copy(g):
        return pltpu.make_async_copy(v_hbm.at[0, pair(g)], v_v.at[pair(g)], sem_v.at[g])

    def wq_copy(g):
        cols = pl.ds(pl.multiple_of(g * 2 * DH, 2 * DH), 2 * DH)
        return pltpu.make_async_copy(wq_hbm.at[:, cols], wq_v.at[g], sem_q.at[g])

    def wo_copy(g):
        src, dst, n = (0, DH, DH) if g == 'first' else (H * DH - DH, H * DH, DH) if g == 'last' \
            else ((2 * g - 1) * DH, 2 * g * DH, 2 * DH)
        al = lambda o: o if isinstance(o, int) else pl.multiple_of(o, DH)
        k = 0 if g == 'first' else NG if g == 'last' else g
        return pltpu.make_async_copy(wo_hbm.at[pl.ds(al(src), n)], wo_v.at[pl.ds(al(dst), n)], sem_o.at[k])

    def m2_copy(j):
        cols = pl.ds(pl.multiple_of(2 * D + j * MC, MC), MC)
        return pltpu.make_async_copy(wm_hbm.at[:, cols], wm2_v.at[j % 2], sem_m2.at[j % 2])

    def q_proj(g, e, i):
        q = jnp.dot(h_v[_t(i), :], wq_v[g, :, e * DH:(e + 1) * DH], preferred_element_type=F32)
        q_v[_t(i), :] = (q * QSCALE).astype(BF16)

    def qk(h, i, ties=()):
        def dot(q, keys):
            return lax.dot_general(q, k_v[h, keys, :], NT_DIMS, preferred_element_type=F32)
        if not ties:
            return dot(q_v[_t(i), :], slice(None))
        q = q_v[_t(i), :].astype(F32)
        return jnp.concatenate(
            [dot(_tie(q, [t for t in ties if t[0] <= r]).astype(BF16), slice(r * 512, (r + 1) * 512))
             for r in range(4)], axis=1)

    def pv(h, s, ties=()):
        m = jnp.max(s, axis=-1, keepdims=True)
        if ties:
            m = jnp.concatenate(
                [jnp.concatenate([_tie(m, [t for t in ties if t[0] <= r])] * 4, axis=1)
                 for r in range(4)], axis=1)
        p = jnp.exp2(s - m)
        l = p[:, 0:128]
        for j in range(1, S // 128):
            l = l + p[:, j * 128:(j + 1) * 128]
        return jnp.dot(p.astype(BF16), v_v[h], preferred_element_type=F32), l

    def out_proj(h, o, l, ties=(), w=None):
        inv = _tie(_recip(_rowsum(l)), ties)
        if w is None:
            w = wo_v[pl.ds(pl.multiple_of((h + 1) * DH, DH), DH), :]
        return jnp.dot((o * inv).astype(BF16), w, preferred_element_type=F32)

    def mod_part(j, e):
        cs = slice(e * DH, (e + 1) * DH)
        mod_v[j, :, cs] = jnp.dot(sc_v[...], wm2_v[j % 2, :, cs], preferred_element_type=F32)[0:8]

    def run_head(g, e):
        h = 2 * g + e
        for tok in BODY_SEQ.split():
            kind, i = tok[0], int(tok[1:])
            if kind == 'Q':
                s = qk(h, i)
            elif kind == 'P':
                os_v[_t(i), :], ls_v[_t(i), :] = pv(h, s)
            elif kind == 'N':
                acc_v[_t(i), :] += out_proj(h - 1, os_v[_t(i), :], ls_v[_t(i), :])
            elif kind == 'Y' and i < NT:
                q_proj(g, e, i)
            else:
                mod_part(g, e)

    def prologue(wm_v, h1_v, sem_m):
        def m_copy(j):
            r = slice(j * DH, (j + 1) * DH)
            return pltpu.make_async_copy(wm_hbm.at[r, 0:2 * D], wm_v.at[r], sem_m.at[j])

        nk = D // DH
        urgent = ([x_copy(i) for i in range(NT)] + [m_copy(j) for j in range(nk)]
                  + [wq_copy(0), wo_copy('first'), m2_copy(0), k_copy(0), v_copy(0)])
        for cp in urgent[:URGENT]:
            cp.start()

        cf = c_ref[...].astype(F32)
        sc = jnp.broadcast_to((cf * jax.nn.sigmoid(cf)).astype(BF16), (16, D))
        sc_v[...] = sc

        @pl.loop(0, NT)
        def _(i):
            x_copy(i).wait()
            acc_v[_dyn(i), :] = _normed(x_v[_dyn(i), :].astype(F32))[0]

        os_v[...] = jnp.zeros((S, DH), F32)
        ls_v[...] = jnp.ones((S, DH), F32)
        wo_v[0:DH, :] = jnp.zeros((DH, D), BF16)
        y = 0.0
        for j in range(nk):
            m_copy(j).wait()
            if j == RELEASE:
                for cp in urgent[URGENT:]:
                    cp.start()
            y = y + jnp.dot(sc[:, j * DH:(j + 1) * DH], wm_v[j * DH:(j + 1) * DH, :],
                            preferred_element_type=F32)[0:8]
        h1_v[0] = _rb(y[:, :D])
        h1_v[1] = 1.0 + _rb(y[:, D:])

        @pl.loop(0, NT)
        def _(i):
            h_v[_dyn(i), :] = (acc_v[_dyn(i), :] * h1_v[1, 0:1, :] + h1_v[0, 0:1, :]).astype(BF16)
            acc_v[_dyn(i), :] = jnp.zeros((TQ, D), F32)

    pl.run_scoped(prologue, pltpu.VMEM((D, 2 * D), BF16), pltpu.VMEM((2, 8, D), F32),
                  pltpu.SemaphoreType.DMA((2 * NM,)))

    def rest(wg_v, wu_v, wd_v, st_v, sem_w, sem_out):
        def w_copies(j):
            c = pl.ds(pl.multiple_of(j * FS, FS), FS)
            return [pltpu.make_async_copy(wg_hbm.at[:, c], wg_v.at[j], sem_w.at[0, j]),
                    pltpu.make_async_copy(wu_hbm.at[:, c], wu_v.at[j], sem_w.at[1, j]),
                    pltpu.make_async_copy(wd_hbm.at[c], wd_v.at[c], sem_w.at[2, j])]

        def body(g, carry):
            for cp in (k_copy(g), v_copy(g), wq_copy(g), m2_copy(g)):
                cp.wait()

            @pl.when(g == 0)
            def _():
                wo_copy('first').wait()

            @pl.when(g > 0)
            def _():
                wo_copy(g).wait()

            @pl.when(g + 1 < NG)
            def _():
                for cp in (k_copy(g + 1), v_copy(g + 1), wq_copy(g + 1), wo_copy(g + 1), m2_copy(g + 1)):
                    cp.start()

            @pl.when(g < F // FS)
            def _():
                for cp in w_copies(g):
                    cp.start()
            run_head(g, 0)
            run_head(g, 1)
            return carry

        wo_copy('last').start()
        lax.fori_loop(0, NG, body, 0)
        wo_copy('last').wait()

        def vec(n):
            return _rb(jnp.concatenate([mod_v[n * NM + j, 0:1, :] for j in range(NM)], axis=1))

        ga, sb, gb = vec(0), vec(1), vec(3)
        cb1 = _rb(1.0 + vec(2))
        wr = wr_ref[...].astype(F32).reshape(1, D)
        wc = cb1 * wr
        wc_sum, sw_sum = _rowsum(wc), _rowsum(sb * wr)
        NEG = -jnp.inf
        out_v = h_v

        def out_copy(n):
            r = pl.ds(pl.multiple_of(n * FG * TQ, FG * TQ), FG * TQ)
            return pltpu.make_async_copy(out_v.at[r], out_hbm.at[0, r], sem_out.at[n])

        gc, gs = gb * cb1, gb * sb

        def rows(i):
            return pl.ds(pl.multiple_of(i * TQ, TQ), TQ)

        def finish(i, top):
            y = out_proj(H - 1, os_v[rows(i), :], ls_v[rows(i), :])
            x1 = x_v[rows(i), :].astype(F32) + ga * (acc_v[rows(i), :] + y)
            x_v[rows(i), :] = x1.astype(BF16)
            xn, mu, rs = _normed(x1, True)
            st_v[0, rows(i), :] = jnp.broadcast_to(mu, (TQ, DH))
            st_v[1, rows(i), :] = jnp.broadcast_to(rs, (TQ, DH))
            outs, rs_, done, rs_full = [], [], [], jnp.broadcast_to(rs, (TQ, DH))
            for e in range(TQ // 8):
                g = slice(8 * e, 8 * e + 8)
                re = rs_full[g]
                if e >= THROTTLE:
                    re = jnp.where(done[e - THROTTLE] < 0.0, 0.0, re)
                xg = (x1[g] - mu[g]) * jnp.concatenate([re] * (D // DH), axis=1)
                if R_MODE == 0:
                    o = x1[g] + (xg * gc + gs)
                    rg = re * (_rowsum(x1[g] * wc) - mu[g] * wc_sum) + sw_sum
                else:
                    h2 = xg * cb1 + sb
                    o = x1[g] + gb * h2
                    rg = _rowsum(h2 * wr)
                if R_MODE == 0:
                    d = o[:, D - DH:]
                else:
                    d = rg
                outs.append(o), rs_.append(rg), done.append(d * d)
            out_v[rows(i), :] = jnp.concatenate(outs, axis=0).astype(BF16)
            m1, m2, k1, k2 = top
            for e in range(TQ // 8):
                re, ke = rs_[e][:, 0:1], i * (TQ // 8) + e
                g1, g2 = re > m1, re > m2
                m2 = jnp.where(g1, m1, jnp.where(g2, re, m2))
                k2 = jnp.where(g1, k1, jnp.where(g2, ke, k2))
                m1 = jnp.where(g1, re, m1)
                k1 = jnp.where(g1, ke, k1)
            return m1, m2, k1, k2

        def finish_group(n, top):
            for e in range(FG):
                top = finish(n * FG + e, top)
            out_copy(n).start()
            return top

        top = lax.fori_loop(0, NT // FG, finish_group, (
            jnp.full((8, 1), NEG, F32), jnp.full((8, 1), NEG, F32),
            jnp.zeros((8, 1), jnp.int32), jnp.ones((8, 1), jnp.int32)))

        m1, m2, k1, k2 = top
        sub = lax.broadcasted_iota(jnp.int32, (8, 1), 0)
        i1, i2 = k1 * 8 + sub, k2 * 8 + sub
        b1 = jnp.max(m1, axis=0, keepdims=True)
        j1 = jnp.min(jnp.where(m1 == b1, i1, S), axis=0, keepdims=True)
        won = i1 == j1
        n1 = jnp.where(won, m2, m1)
        ni = jnp.where(won, i2, i1)
        b2 = jnp.max(n1, axis=0, keepdims=True)
        j2 = jnp.min(jnp.where((n1 == b2) & (ni != j1), ni, S), axis=0, keepdims=True)
        idx1 = jnp.clip(j1[0, 0], 0, S - 1)
        idx2 = jnp.clip(j2[0, 0], 0, S - 1)
        rid = lax.broadcasted_iota(jnp.int32, (16, D), 0)

        def base_of(idx):
            return pl.multiple_of((idx // 16) * 16, 16)

        def h2_row(idx):
            base = base_of(idx)
            blk = x_v[pl.ds(base, 16), :].astype(F32)
            x1 = jnp.sum(jnp.where(rid == idx - base, blk, 0.0), axis=0, keepdims=True)
            mu, rs = st_v[0, pl.ds(idx, 1), :][:, 0:1], st_v[1, pl.ds(idx, 1), :][:, 0:1]
            return (x1 - mu) * rs * cb1 + sb

        h2a, h2b = h2_row(idx1), h2_row(idx2)
        xs = jnp.where(rid == 0, h2a, jnp.where(rid == 1, h2b, 0.0)).astype(BF16)
        for j in range(F // FS):
            for cp in w_copies(j):
                cp.wait()
        FC = FS
        acts = []
        for j in range(F // FC):
            cs = slice(j * FC, (j + 1) * FC)
            g = jnp.dot(xs, wg_v[j], preferred_element_type=F32)
            u = jnp.dot(xs, wu_v[j], preferred_element_type=F32)
            acts.append((g * jax.nn.sigmoid(g) * u).astype(BF16))
        y = None
        for j, a in enumerate(acts):
            yj = jnp.dot(a, wd_v[j * FC:(j + 1) * FC, :], preferred_element_type=F32)
            y = yj if y is None else y + yj
        ua = gb * (y[0:1] * jax.nn.sigmoid(_rb(b1)))
        ub = gb * (y[1:2] * jax.nn.sigmoid(_rb(b2)))

        for n in range(NT // FG):
            out_copy(n).wait()

        def patch(idx, row):
            base = base_of(idx)
            blk = out_v[pl.ds(base, 16), :].astype(F32)
            out_v[pl.ds(base, 16), :] = jnp.where(rid == idx - base, blk + row, blk).astype(BF16)
            return base

        def patch_copy(base, k):
            return pltpu.make_async_copy(out_v.at[pl.ds(base, 16)],
                                         out_hbm.at[0, pl.ds(base, 16)], sem_out.at[k])

        p1 = patch(idx1, ua)
        p2 = patch(idx2, ub)
        patch_copy(p1, 0).start()

        @pl.when(p1 != p2)
        def _():
            patch_copy(p2, 1).start()
            patch_copy(p2, 1).wait()
        patch_copy(p1, 0).wait()

    pl.run_scoped(
        rest,
        pltpu.VMEM((F // FS, D, FS), BF16),
        pltpu.VMEM((F // FS, D, FS), BF16),
        pltpu.VMEM((F, D), BF16),
        pltpu.VMEM((2, S, DH), F32),
        pltpu.SemaphoreType.DMA((3, F // FS)),
        pltpu.SemaphoreType.DMA((NT,)),
    )


@jax.jit
def pallas_adaLN_cond__mha_block_cached__moe_arch_mod__prompt_kernel(
    A_x: jax.Array,
    A_k_cache: jax.Array,
    A_v_cache: jax.Array,
    A_wq: jax.Array,
    A_wo: jax.Array,
    B_x: jax.Array,
    B_w_r: jax.Array,
    B_w_gate: jax.Array,
    B_w_up: jax.Array,
    B_w_down: jax.Array,
    c: jax.Array,
    w_mod: jax.Array,
):
    del B_x
    hbm = pl.BlockSpec(memory_space=pl.ANY)
    vmem = pl.BlockSpec(memory_space=pltpu.VMEM)
    return pl.pallas_call(
        _kernel,
        out_shape=jax.ShapeDtypeStruct((1, S, D), BF16),
        in_specs=[vmem, vmem] + [hbm] * 9,
        out_specs=hbm,
        scratch_shapes=[
            pltpu.VMEM((S, D), BF16),
            pltpu.VMEM((S, D), BF16),
            pltpu.VMEM((H, S, DH), BF16),
            pltpu.VMEM((H, S, DH), BF16),
            pltpu.VMEM((NG, D, 2 * DH), BF16),
            pltpu.VMEM((H * DH + DH, D), BF16),
            pltpu.VMEM((S, D), F32),
            pltpu.VMEM((S, DH), F32),
            pltpu.VMEM((S, DH), F32),
            pltpu.VMEM((S, DH), BF16),
            pltpu.VMEM((16, D), BF16),
            pltpu.VMEM((4 * NM, 8, MC), F32),
            pltpu.VMEM((2, D, MC), BF16),
            pltpu.SemaphoreType.DMA((NT,)),
            pltpu.SemaphoreType.DMA((NG,)),
            pltpu.SemaphoreType.DMA((NG,)),
            pltpu.SemaphoreType.DMA((NG,)),
            pltpu.SemaphoreType.DMA((NG + 1,)),
            pltpu.SemaphoreType.DMA((2,)),
        ],
        compiler_params=pltpu.CompilerParams(vmem_limit_bytes=127 * 1024 * 1024),
    )(c, B_w_r, A_x, A_k_cache, A_v_cache, A_wq, A_wo,
      B_w_gate, B_w_up, B_w_down, w_mod)
```
